```python
import os as _os
_os.environ.setdefault("JAX_PLATFORMS", "cpu")
import jax
import jax.numpy as jnp

def _softmax(x, axis=-1):
    return jax.nn.softmax(x, axis=axis)
def _gelu(x):
    return jax.nn.gelu(x, approximate=True)
def _silu(x):
    return jax.nn.silu(x)
def _sigmoid(x):
    return jax.nn.sigmoid(x)
def _layernorm(x, axis=-1, eps=1e-5):
    m = jnp.mean(x, axis=axis, keepdims=True)
    v = jnp.var(x, axis=axis, keepdims=True)
    return (x - m) / jnp.sqrt(v + eps)
def _scatter_add(tgt, idx, src, axis=0):
    return tgt.at[idx].add(src)
def _segment_sum(src, seg, n):
    return jax.ops.segment_sum(src, seg, n)
class _Rng:
    def __init__(self, key):
        self._k = key
    def _next(self):
        self._k, sub = jax.random.split(self._k)
        return sub
    def normal(self, shape):
        return jax.random.normal(self._next(), shape, dtype=jnp.bfloat16)
    def randint(self, lo, hi, shape):
        return jax.random.randint(self._next(), shape, lo, hi, dtype=jnp.int32)
    def uniform(self, shape, lo=0.0, hi=1.0):
        return jax.random.uniform(self._next(), shape, jnp.bfloat16, lo, hi)
    def permutation(self, n):
        return jax.random.permutation(self._next(), n)


kernel_name = 'standalone__channel_attn_cbam__vision'

def setup_inputs():
    _rng = _Rng(jax.random.key(int.from_bytes(__import__("os").urandom(4), "little")))
    _w = (lambda a: (lambda t: t.astype(jnp.bfloat16) if jnp.issubdtype(t.dtype, jnp.floating) else t)(jnp.asarray(a)))
    H = W = 224
    C = 192
    r = max(C // 4, 1)
    return {
        "x": _w((lambda *s: _rng.normal(s) * 0.2)(1, H, W, C) + (lambda *s: _rng.normal(s) * 0.2)(1, 1, 1, C) * 2.0),
        "w1": _w((lambda *s: _rng.normal(s) * 0.2)(C, r)),
        "w2": _w((lambda *s: _rng.normal(s) * 0.2)(r, C)),
    }

def reference(x, w1, w2):
    B, H, W, C = x.shape
    xf = x.reshape(B, H * W, C)
    gap = jnp.mean(xf, 1)
    gmp = jnp.amax(xf, 1)
    h_a = gap @ w1
    h_a = h_a * (lambda x, dt: x.astype(dt))(h_a > 0, h_a.dtype)
    h_m = gmp @ w1
    h_m = h_m * (lambda x, dt: x.astype(dt))(h_m > 0, h_m.dtype)
    scale = _sigmoid(h_a @ w2 + h_m @ w2)
    return x * scale[:, None, None, :]
```

```python
import jax
import jax.numpy as jnp
from jax import lax
import jax.experimental.pallas as pl
import jax.experimental.pallas.tpu as pltpu

_NS = 8
_CB = 16
_NSEM = 4


def _cbam_kernel(x_hbm, w1t_hbm, w2_hbm, o_hbm,
                 xbuf, obuf, w1t_v, w2_v, acc_s, acc_m, scale_ref,
                 in_sems, out_sem):
    NS, G, NCB, CB, W = x_hbm.shape
    C = NCB * CB
    HW = NS * G * W
    hs = NS // 2

    def start_chunk(g, slot):
        for cb in range(NCB):
            for half in range(2):
                pltpu.make_async_copy(
                    x_hbm.at[pl.ds(half * hs, hs), g, cb],
                    xbuf.at[g, cb, pl.ds(half * hs, hs)],
                    in_sems.at[slot],
                ).start(priority=half)

    def wait_chunk(g, slot):
        pltpu.make_async_copy(xbuf.at[g], xbuf.at[g], in_sems.at[slot]).wait()

    for g in range(_NSEM):
        start_chunk(g, g)
    cw1 = pltpu.make_async_copy(w1t_hbm, w1t_v, out_sem)
    cw2 = pltpu.make_async_copy(w2_hbm, w2_v, out_sem)
    cw1.start()
    cw2.start()

    acc_s[...] = jnp.zeros(acc_s.shape, jnp.float32)
    acc_m[...] = jnp.full(acc_m.shape, -jnp.inf, jnp.float32)

    def body1(g, carry):
        slot = g % _NSEM
        wait_chunk(g, slot)

        @pl.when(g + _NSEM < G)
        def _():
            start_chunk(g + _NSEM, slot)

        for cb in range(NCB):
            xs = xbuf[g, cb].astype(jnp.float32)
            acc_s[cb] += jnp.sum(xs, axis=0)
            acc_m[cb] = jnp.maximum(acc_m[cb], jnp.max(xs, axis=0))
        return carry

    lax.fori_loop(0, G, body1, 0)
    cw1.wait()
    cw2.wait()

    s_all = acc_s[...].reshape(C, W)
    m_all = acc_m[...].reshape(C, W)
    gap = jnp.sum(s_all, axis=1, keepdims=True) * (1.0 / HW)
    gmp = jnp.max(m_all, axis=1, keepdims=True)
    gcat = jnp.concatenate(
        [jnp.broadcast_to(gap, (C, 128)), jnp.broadcast_to(gmp, (C, 128))], axis=1
    ).astype(jnp.bfloat16)
    h = jnp.dot(w1t_v[...], gcat, preferred_element_type=jnp.float32)
    h = h.astype(jnp.bfloat16).astype(jnp.float32)
    h = jnp.maximum(h, 0.0).astype(jnp.bfloat16)
    z = lax.dot_general(w2_v[...], h, (((0,), (0,)), ((), ())),
                        preferred_element_type=jnp.float32)
    z = z.astype(jnp.bfloat16).astype(jnp.float32)
    zz = (z[:, :128] + z[:, 128:]).astype(jnp.bfloat16).astype(jnp.float32)
    sc = jax.nn.sigmoid(zz).astype(jnp.bfloat16).astype(jnp.float32)
    scale_ref[:, 0:128] = sc
    scale_ref[:, 128:W] = sc[:, : W - 128]

    def body2(g, carry):
        for cb in range(NCB):
            xs = xbuf[g, cb].astype(jnp.float32)
            s = scale_ref[cb * CB:(cb + 1) * CB, :]
            obuf[g, cb] = (xs * s[None]).astype(jnp.bfloat16)
            pltpu.make_async_copy(obuf.at[g, cb], o_hbm.at[:, g, cb], out_sem).start()
        return carry

    lax.fori_loop(0, G, body2, 0)
    pltpu.make_async_copy(obuf, obuf, out_sem).wait()


@jax.jit
def pallas_standalone__channel_attn_cbam__vision_kernel(
    x: jax.Array,
    w1: jax.Array,
    w2: jax.Array,
):
    B, H, W, C = x.shape
    assert B == 1 and H % _NS == 0 and C % _CB == 0 and 128 < W <= 256
    G = H // _NS
    NCB = C // _CB
    R = w1.shape[1]
    xt = jnp.transpose(x, (0, 1, 3, 2)).reshape(_NS, G, NCB, _CB, W)
    w1t = w1.T
    out = pl.pallas_call(
        _cbam_kernel,
        out_shape=jax.ShapeDtypeStruct((_NS, G, NCB, _CB, W), x.dtype),
        in_specs=[
            pl.BlockSpec(memory_space=pl.ANY),
            pl.BlockSpec(memory_space=pl.ANY),
            pl.BlockSpec(memory_space=pl.ANY),
        ],
        out_specs=pl.BlockSpec(memory_space=pl.ANY),
        scratch_shapes=[
            pltpu.VMEM((G, NCB, _NS, _CB, W), x.dtype),
            pltpu.VMEM((G, NCB, _NS, _CB, W), x.dtype),
            pltpu.VMEM((R, C), w1.dtype),
            pltpu.VMEM((R, C), w2.dtype),
            pltpu.VMEM((NCB, _CB, W), jnp.float32),
            pltpu.VMEM((NCB, _CB, W), jnp.float32),
            pltpu.VMEM((C, W), jnp.float32),
            pltpu.SemaphoreType.DMA((_NSEM,)),
            pltpu.SemaphoreType.DMA(()),
        ],
        compiler_params=pltpu.CompilerParams(vmem_limit_bytes=100 * 1024 * 1024),
    )(xt, w1t, w2)
    return jnp.transpose(out.reshape(B, H, C, W), (0, 1, 3, 2))
```

```python
import jax
import jax.numpy as jnp
from jax import lax
import jax.experimental.pallas as pl
import jax.experimental.pallas.tpu as pltpu

_F32 = jnp.float32
_BF16 = jnp.bfloat16

_CB = 16
_NS = 8
_K = 4
_L = 2
_T = 2
_HEAD = 16
_AW = 7
_RW = 3
_E = 5
_TAIL = (((0, 3),), ((3, 6),), ((6, 9),), ((9, 11), (11, 12)))
_GROUPS = tuple(grp for blk in _TAIL for grp in blk)


def _tree(op, xs):
    xs = list(xs)
    while len(xs) > 1:
        nxt = [op(xs[i], xs[i + 1]) for i in range(0, len(xs) - 1, 2)]
        if len(xs) % 2:
            nxt.append(xs[-1])
        xs = nxt
    return xs[0]


def _wait_for(ref, sem):
    pltpu.make_async_copy(ref, ref, sem).wait()


def _body(x_hbm, w1t_hbm, w2_hbm, o_hbm,
          xbuf, obuf, w1t_v, w2_v, w1d, w2d, acc_s, acc_m, scale_ref, pad_a, pad_b,
          out_sem, sem_a, sem_b, tail_a, tail_b, w_sem):
    NS, G, NCB, CB, W = x_hbm.shape
    C = NCB * CB
    R = w1t_v.shape[0]
    HW = NS * G * W
    hs = NS // 2
    GM = G - _T
    per_batch = NCB // _T
    n_grp = len(_GROUPS)

    def start_one(g, half, cb, sem):
        prio = half
        if isinstance(g, int) and g * NCB + cb < _HEAD:
            prio = 1
        pltpu.make_async_copy(
            x_hbm.at[pl.ds(half * hs, hs), g, cb], xbuf.at[g, half, cb], sem
        ).start(priority=prio)

    def start_chunk(g, slot):
        for cb in range(NCB):
            start_one(g, 0, cb, sem_a.at[slot])
            start_one(g, 1, cb, sem_b.at[slot])

    def wait_half(g, half):
        _wait_for(xbuf.at[g, half], (sem_a, sem_b)[half].at[g % _K])

    def tail_b_sem(g, cb):
        if cb == NCB - 1 and g == G - 1:
            return tail_b.at[n_grp]
        (t,) = [i for i, (lo, hi) in enumerate(_GROUPS) if lo <= cb < hi]
        return tail_b.at[t]

    def start_tail_batch(j):
        for cb in range(j * per_batch, (j + 1) * per_batch):
            for g in range(GM, G):
                start_one(g, 0, cb, tail_a.at[j])
                start_one(g, 1, cb, tail_b_sem(g, cb))

    for g in range(_K):
        start_chunk(g, g)
    cw1 = pltpu.make_async_copy(w1t_hbm, w1t_v, w_sem)
    cw2 = pltpu.make_async_copy(w2_hbm, w2_v, w_sem)
    cw1.start()
    cw2.start()

    acc_s[...] = jnp.zeros(acc_s.shape, _F32)
    acc_m[...] = jnp.full(acc_m.shape, -jnp.inf, _F32)
    pad_a[...] = jnp.zeros(pad_a.shape, _F32)

    def red(pieces, cb, s0=None, m0=None):
        xs = [xbuf[g, half, cb, s].astype(_F32) for (g, half) in pieces for s in range(hs)]
        s0 = acc_s[cb] if s0 is None else s0
        m0 = acc_m[cb] if m0 is None else m0
        return s0 + _tree(jnp.add, xs), jnp.maximum(m0, _tree(jnp.maximum, xs))

    def accum(pieces, cbs):
        for cb in cbs:
            s, m = red(pieces, cb)
            acc_s[cb] = s
            acc_m[cb] = m

    all_cb = range(NCB)

    def body_head(g, carry):
        wait_half(g, 0)
        accum([(g, 0)], all_cb)
        return carry

    lax.fori_loop(0, _L, body_head, 0)

    def body_main(g, carry):
        wait_half(g, 1)
        start_chunk(g + _K, g % _K)
        accum([(g, 1)], all_cb)
        wait_half(g + _L, 0)
        accum([(g + _L, 0)], all_cb)
        return carry

    lax.fori_loop(0, GM - _K, body_main, 0)

    def do_first_half(a):
        if a < GM:
            wait_half(a, 0)
            accum([(a, 0)], all_cb)
        elif a - GM < _T:
            j = a - GM
            _wait_for(xbuf.at[pl.ds(GM, _T), 0, pl.ds(j * per_batch, per_batch)], tail_a.at[j])
            accum([(g, 0) for g in range(GM, G)],
                  range(j * per_batch, (j + 1) * per_batch))

    fence = pltpu.make_async_copy(pad_a, pad_b, w_sem)
    for g in range(GM - _K, GM):
        wait_half(g, 1)
        j = g - (GM - _K)
        if j < _T:
            start_tail_batch(j)
        if j == 0:
            cw1.wait()
            cw2.wait()
            fence.start()
            zpad = jnp.zeros((64 - R, C), _F32)
            a = w1t_v[...].astype(_F32)
            w1d[...] = jnp.concatenate([a, zpad, a, zpad], axis=0).T
            b = w2_v[...].astype(_F32)
            w2d[...] = jnp.concatenate([b, zpad, b, zpad], axis=0).T
        accum([(g, 1)], all_cb)
        do_first_half(g + _L)
    for a in range(GM + _L, GM + _T):
        do_first_half(a)

    lane = lax.broadcasted_iota(jnp.int32, (CB, 128), 1)
    pacc = jnp.zeros((8, 128), _F32)
    tail_pieces = [(g, 1) for g in range(GM, G)]
    t = 0
    for blk in _TAIL:
        totals = []
        for (lo, hi) in blk:
            last = hi == NCB
            if last:
                if hi - lo > 1:
                    _wait_for(xbuf.at[pl.ds(GM, _T), 1, pl.ds(lo, hi - 1 - lo)], tail_b.at[t])
                if _T > 1:
                    _wait_for(xbuf.at[pl.ds(GM, _T - 1), 1, NCB - 1], tail_b.at[t])
            else:
                _wait_for(xbuf.at[pl.ds(GM, _T), 1, pl.ds(lo, hi - lo)], tail_b.at[t])
            t += 1
            for cb in range(lo, hi):
                if last and cb == NCB - 1:
                    s, m = red(tail_pieces[:-1], cb) if _T > 1 else (acc_s[cb], acc_m[cb])
                    _wait_for(xbuf.at[G - 1, 1, cb], tail_b.at[n_grp])
                    totals.append((cb, red(tail_pieces[-1:], cb, s, m)))
                else:
                    totals.append((cb, red(tail_pieces, cb)))
        for cb, (s, m) in totals:
            gap = jnp.sum(s, axis=1, keepdims=True) * (1.0 / HW)
            gap = gap.astype(_BF16).astype(_F32)
            gmp = jnp.max(m, axis=1, keepdims=True)
            p = w1d[cb * CB:(cb + 1) * CB, :] * jnp.where(lane < 64, gap, gmp)
            pacc = pacc + _tree(jnp.add, [p[i * 8:(i + 1) * 8] for i in range(CB // 8)])

    h = jnp.sum(pacc, axis=0, keepdims=True)
    h = jnp.maximum(h.astype(_BF16).astype(_F32), 0.0)

    GW = (NS * G) // _AW
    NP = NCB // _RW

    def scale_of(cb):
        z = jnp.sum(w2d[cb * CB:(cb + 1) * CB, :] * h, axis=1, keepdims=True)
        sc = 0.5 * jnp.tanh(0.5 * z) + 0.5
        return jnp.broadcast_to(sc.astype(_BF16).astype(_F32), (CB, 128))

    def load_scale(cb):
        return scale_ref[cb * CB:(cb + 1) * CB, :]

    def scale_rows(gw, cb, s128):
        s = jnp.concatenate([s128, s128[:, :W - 128]], axis=1)
        p, r = divmod(cb, _RW)
        for a in range(_AW):
            row = GW * a + gw
            stream = row // G
            g = row - stream * G
            xs = xbuf[g, stream // hs, cb, stream % hs].astype(_F32)
            obuf[gw, p, a, pl.ds(r * CB, CB)] = (xs * s).astype(_BF16)

    def start_out(gw, p, lo, n):
        pltpu.make_async_copy(
            obuf.at[gw, p, :, pl.ds(lo * CB, n * CB)],
            o_hbm.at[:, gw, p, pl.ds(lo * CB, n * CB)],
            out_sem,
        ).start()

    s_first = scale_of(0)
    for gw in range(_E):
        scale_rows(gw, 0, s_first)
        start_out(gw, 0, 0, 1)
    fence.wait()
    scale_ref[0:CB, :] = s_first
    for cb in range(1, NCB):
        scale_ref[cb * CB:(cb + 1) * CB, :] = scale_of(cb)

    def out_rows(skip_first):
        def body(gw, carry):
            for p in range(NP):
                lo = 1 if (skip_first and p == 0) else 0
                if lo == _RW:
                    continue
                for r in range(lo, _RW):
                    scale_rows(gw, p * _RW + r, load_scale(p * _RW + r))
                start_out(gw, p, lo, _RW - lo)
            return carry
        return body

    lax.fori_loop(0, _E, out_rows(True), 0)
    lax.fori_loop(_E, GW, out_rows(False), 0)


def _kernel(x_hbm, w1t_hbm, w2_hbm, o_hbm, *scratch):
    out_sem = scratch[-1]

    def scoped(*sems):
        _body(x_hbm, w1t_hbm, w2_hbm, o_hbm, *scratch, *sems)

    pl.run_scoped(
        scoped,
        pltpu.SemaphoreType.DMA((_K,)),
        pltpu.SemaphoreType.DMA((_K,)),
        pltpu.SemaphoreType.DMA((_T,)),
        pltpu.SemaphoreType.DMA((len(_GROUPS) + 1,)),
        pltpu.SemaphoreType.DMA(()),
    )
    _wait_for(o_hbm, out_sem)


@jax.jit
def pallas_standalone__channel_attn_cbam__vision_kernel(
    x: jax.Array,
    w1: jax.Array,
    w2: jax.Array,
):
    B, H, W, C = x.shape
    R = w1.shape[1]
    G = H // _NS
    NCB = C // _CB
    assert B == 1 and H % _NS == 0 and H % _AW == 0 and C % (_CB * _RW) == 0
    assert NCB == _GROUPS[-1][1] and NCB % _T == 0 and G >= _K + _T + _L
    assert 128 < W <= 256 and R <= 64 and R % 8 == 0

    xt = jnp.transpose(x, (0, 1, 3, 2)).reshape(_NS, G, NCB, _CB, W)
    w1t = w1.T
    out = pl.pallas_call(
        _kernel,
        out_shape=jax.ShapeDtypeStruct((_AW, H // _AW, NCB // _RW, _RW * _CB, W), x.dtype),
        in_specs=[pl.BlockSpec(memory_space=pl.ANY)] * 3,
        out_specs=pl.BlockSpec(memory_space=pl.ANY),
        scratch_shapes=[
            pltpu.VMEM((G, 2, NCB, _NS // 2, _CB, W), x.dtype),
            pltpu.VMEM((H // _AW, NCB // _RW, _AW, _RW * _CB, W), x.dtype),
            pltpu.VMEM((R, C), w1.dtype),
            pltpu.VMEM((R, C), w2.dtype),
            pltpu.VMEM((C, 128), _F32),
            pltpu.VMEM((C, 128), _F32),
            pltpu.VMEM((NCB, _CB, W), _F32),
            pltpu.VMEM((NCB, _CB, W), _F32),
            pltpu.VMEM((C, 128), _F32),
            pltpu.VMEM((8, 128), _F32),
            pltpu.VMEM((8, 128), _F32),
            pltpu.SemaphoreType.DMA(()),
        ],
        compiler_params=pltpu.CompilerParams(vmem_limit_bytes=100 * 1024 * 1024),
    )(xt, w1t, w2)
    return jnp.transpose(out.reshape(B, H, C, W), (0, 1, 3, 2))
```

```python
import jax
import jax.numpy as jnp
from jax import lax
import jax.experimental.pallas as pl
import jax.experimental.pallas.tpu as pltpu

_F32 = jnp.float32
_BF16 = jnp.bfloat16

_CB = 16
_NS = 7
_S0 = 3
_K = 4
_L = 2
_T = 2
_HEAD = 14
_RW = 2
_E = 4
_TAIL = (((0, 3),), ((3, 6),), ((6, 9),), ((9, 11), (11, 12)))
_GROUPS = tuple(grp for blk in _TAIL for grp in blk)


def _tree(op, xs):
    xs = list(xs)
    while len(xs) > 1:
        nxt = [op(xs[i], xs[i + 1]) for i in range(0, len(xs) - 1, 2)]
        if len(xs) % 2:
            nxt.append(xs[-1])
        xs = nxt
    return xs[0]


def _wait_for(ref, sem):
    pltpu.make_async_copy(ref, ref, sem).wait()


def _body(x_hbm, w1t_hbm, w2_hbm, o_hbm,
          xbuf, obuf, w1t_v, w2_v, w1d, w2d, acc_s, acc_m, scale_ref, pad_a, pad_b,
          out_sem, sem_a, sem_b, tail_a, tail_b, w_sem):
    NS, G, NCB, CB, W = x_hbm.shape
    C = NCB * CB
    R = w1t_v.shape[0]
    HW = NS * G * W
    parts = ((0, _S0), (_S0, NS - _S0))
    GM = G - _T
    per_batch = NCB // _T
    n_grp = len(_GROUPS)

    def start_one(g, half, cb, sem):
        prio = half
        if isinstance(g, int) and g * NCB + cb < _HEAD:
            prio = 1
        s0, n = parts[half]
        pltpu.make_async_copy(
            x_hbm.at[pl.ds(s0, n), g, cb], xbuf.at[g, cb, pl.ds(s0, n)], sem
        ).start(priority=prio)

    def start_chunk(g, slot):
        for cb in range(NCB):
            start_one(g, 0, cb, sem_a.at[slot])
            start_one(g, 1, cb, sem_b.at[slot])

    def wait_half(g, half):
        _wait_for(xbuf.at[g, :, pl.ds(*parts[half])], (sem_a, sem_b)[half].at[g % _K])

    def tail_b_sem(g, cb):
        if cb == NCB - 1 and g == G - 1:
            return tail_b.at[n_grp]
        (t,) = [i for i, (lo, hi) in enumerate(_GROUPS) if lo <= cb < hi]
        return tail_b.at[t]

    def start_tail_batch(j):
        for cb in range(j * per_batch, (j + 1) * per_batch):
            for g in range(GM, G):
                start_one(g, 0, cb, tail_a.at[j])
                start_one(g, 1, cb, tail_b_sem(g, cb))

    for g in range(_K):
        start_chunk(g, g)
    cw1 = pltpu.make_async_copy(w1t_hbm, w1t_v, w_sem)
    cw2 = pltpu.make_async_copy(w2_hbm, w2_v, w_sem)
    cw1.start()
    cw2.start()

    acc_s[...] = jnp.zeros(acc_s.shape, _F32)
    acc_m[...] = jnp.full(acc_m.shape, -jnp.inf, _F32)
    pad_a[...] = jnp.zeros(pad_a.shape, _F32)

    def red(pieces, cb, s0=None, m0=None):
        xs = [xbuf[g, cb, s].astype(_F32) for (g, half) in pieces
              for s in range(parts[half][0], sum(parts[half]))]
        s0 = acc_s[cb] if s0 is None else s0
        m0 = acc_m[cb] if m0 is None else m0
        return s0 + _tree(jnp.add, xs), jnp.maximum(m0, _tree(jnp.maximum, xs))

    def accum(pieces, cbs):
        for cb in cbs:
            s, m = red(pieces, cb)
            acc_s[cb] = s
            acc_m[cb] = m

    all_cb = range(NCB)

    def body_head(g, carry):
        wait_half(g, 0)
        accum([(g, 0)], all_cb)
        return carry

    lax.fori_loop(0, _L, body_head, 0)

    def body_main(g, carry):
        wait_half(g, 1)
        start_chunk(g + _K, g % _K)
        accum([(g, 1)], all_cb)
        wait_half(g + _L, 0)
        accum([(g + _L, 0)], all_cb)
        return carry

    lax.fori_loop(0, GM - _K, body_main, 0)

    def do_first_half(a):
        if a < GM:
            wait_half(a, 0)
            accum([(a, 0)], all_cb)
        elif a - GM < _T:
            j = a - GM
            _wait_for(xbuf.at[pl.ds(GM, _T), pl.ds(j * per_batch, per_batch), pl.ds(*parts[0])],
                      tail_a.at[j])
            accum([(g, 0) for g in range(GM, G)],
                  range(j * per_batch, (j + 1) * per_batch))

    fence = pltpu.make_async_copy(pad_a, pad_b, w_sem)
    for g in range(GM - _K, GM):
        wait_half(g, 1)
        j = g - (GM - _K)
        if j < _T:
            start_tail_batch(j)
        if j == 0:
            cw1.wait()
            cw2.wait()
            fence.start()
            zpad = jnp.zeros((64 - R, C), _F32)
            a = w1t_v[...].astype(_F32)
            w1d[...] = jnp.concatenate([a, zpad, a, zpad], axis=0).T
            b = w2_v[...].astype(_F32)
            w2d[...] = jnp.concatenate([b, zpad, b, zpad], axis=0).T
        accum([(g, 1)], all_cb)
        do_first_half(g + _L)
    for a in range(GM + _L, GM + _T):
        do_first_half(a)

    lane = lax.broadcasted_iota(jnp.int32, (CB, 128), 1)
    pacc = jnp.zeros((8, 128), _F32)
    tail_pieces = [(g, 1) for g in range(GM, G)]
    t = 0
    for blk in _TAIL:
        totals = []
        for (lo, hi) in blk:
            last = hi == NCB
            if last:
                if hi - lo > 1:
                    _wait_for(xbuf.at[pl.ds(GM, _T), pl.ds(lo, hi - 1 - lo), pl.ds(*parts[1])],
                              tail_b.at[t])
                if _T > 1:
                    _wait_for(xbuf.at[pl.ds(GM, _T - 1), NCB - 1, pl.ds(*parts[1])], tail_b.at[t])
            else:
                _wait_for(xbuf.at[pl.ds(GM, _T), pl.ds(lo, hi - lo), pl.ds(*parts[1])],
                          tail_b.at[t])
            t += 1
            for cb in range(lo, hi):
                if last and cb == NCB - 1:
                    s, m = red(tail_pieces[:-1], cb) if _T > 1 else (acc_s[cb], acc_m[cb])
                    _wait_for(xbuf.at[G - 1, cb, pl.ds(*parts[1])], tail_b.at[n_grp])
                    totals.append((cb, red(tail_pieces[-1:], cb, s, m)))
                else:
                    totals.append((cb, red(tail_pieces, cb)))
        for cb, (s, m) in totals:
            gap = jnp.sum(s, axis=1, keepdims=True) * (1.0 / HW)
            gap = gap.astype(_BF16).astype(_F32)
            gmp = jnp.max(m, axis=1, keepdims=True)
            p = w1d[cb * CB:(cb + 1) * CB, :] * jnp.where(lane < 64, gap, gmp)
            pacc = pacc + _tree(jnp.add, [p[i * 8:(i + 1) * 8] for i in range(CB // 8)])

    h = jnp.sum(pacc, axis=0, keepdims=True)
    h = jnp.maximum(h.astype(_BF16).astype(_F32), 0.0)

    NP = NCB // _RW

    def scale_of(cb):
        z = jnp.sum(w2d[cb * CB:(cb + 1) * CB, :] * h, axis=1, keepdims=True)
        sc = 0.5 * jnp.tanh(0.5 * z) + 0.5
        return jnp.broadcast_to(sc.astype(_BF16).astype(_F32), (CB, 128))

    def load_scale(cb):
        return scale_ref[cb * CB:(cb + 1) * CB, :]

    def scale_rows(gw, cb, s128):
        s = jnp.concatenate([s128, s128[:, :W - 128]], axis=1)
        p, r = divmod(cb, _RW)
        xs = xbuf[gw, cb].astype(_F32)
        obuf[gw, p, :, pl.ds(r * CB, CB)] = (xs * s[None]).astype(_BF16)

    def start_out(gw, p, lo, n):
        pltpu.make_async_copy(
            obuf.at[gw, p, :, pl.ds(lo * CB, n * CB)],
            o_hbm.at[:, gw, p, pl.ds(lo * CB, n * CB)],
            out_sem,
        ).start()

    s_first = scale_of(0)
    for gw in range(_E):
        scale_rows(gw, 0, s_first)
        start_out(gw, 0, 0, 1)
    fence.wait()
    scale_ref[0:CB, :] = s_first
    for cb in range(1, NCB):
        scale_ref[cb * CB:(cb + 1) * CB, :] = scale_of(cb)

    def out_rows(skip_first):
        def body(gw, carry):
            for p in range(NP):
                lo = 1 if (skip_first and p == 0) else 0
                if lo == _RW:
                    continue
                for r in range(lo, _RW):
                    scale_rows(gw, p * _RW + r, load_scale(p * _RW + r))
                start_out(gw, p, lo, _RW - lo)
            return carry
        return body

    lax.fori_loop(0, _E, out_rows(True), 0)
    lax.fori_loop(_E, G, out_rows(False), 0)


def _kernel(x_hbm, w1t_hbm, w2_hbm, o_hbm, *scratch):
    out_sem = scratch[-1]

    def scoped(*sems):
        _body(x_hbm, w1t_hbm, w2_hbm, o_hbm, *scratch, *sems)

    pl.run_scoped(
        scoped,
        pltpu.SemaphoreType.DMA((_K,)),
        pltpu.SemaphoreType.DMA((_K,)),
        pltpu.SemaphoreType.DMA((_T,)),
        pltpu.SemaphoreType.DMA((len(_GROUPS) + 1,)),
        pltpu.SemaphoreType.DMA(()),
    )
    _wait_for(o_hbm, out_sem)


@jax.jit
def pallas_standalone__channel_attn_cbam__vision_kernel(
    x: jax.Array,
    w1: jax.Array,
    w2: jax.Array,
):
    B, H, W, C = x.shape
    R = w1.shape[1]
    G = H // _NS
    NCB = C // _CB
    assert B == 1 and H % _NS == 0 and C % (_CB * _RW) == 0
    assert NCB == _GROUPS[-1][1] and NCB % _T == 0 and G >= _K + _T + _L
    assert 128 < W <= 256 and R < 64 and R % 8 == 0

    xt = jnp.transpose(x, (0, 1, 3, 2)).reshape(_NS, G, NCB, _CB, W)
    w1t = w1.T
    out = pl.pallas_call(
        _kernel,
        out_shape=jax.ShapeDtypeStruct((_NS, G, NCB // _RW, _RW * _CB, W), x.dtype),
        in_specs=[pl.BlockSpec(memory_space=pl.ANY)] * 3,
        out_specs=pl.BlockSpec(memory_space=pl.ANY),
        scratch_shapes=[
            pltpu.VMEM((G, NCB, _NS, _CB, W), x.dtype),
            pltpu.VMEM((G, NCB // _RW, _NS, _RW * _CB, W), x.dtype),
            pltpu.VMEM((R, C), w1.dtype),
            pltpu.VMEM((R, C), w2.dtype),
            pltpu.VMEM((C, 128), _F32),
            pltpu.VMEM((C, 128), _F32),
            pltpu.VMEM((NCB, _CB, W), _F32),
            pltpu.VMEM((NCB, _CB, W), _F32),
            pltpu.VMEM((C, 128), _F32),
            pltpu.VMEM((8, 128), _F32),
            pltpu.VMEM((8, 128), _F32),
            pltpu.SemaphoreType.DMA(()),
        ],
        compiler_params=pltpu.CompilerParams(vmem_limit_bytes=100 * 1024 * 1024),
    )(xt, w1t, w2)
    return jnp.transpose(out.reshape(B, H, C, W), (0, 1, 3, 2))
```
